```python
import os as _os
_os.environ.setdefault("JAX_PLATFORMS", "cpu")
import jax
import jax.numpy as jnp

def _softmax(x, axis=-1):
    return jax.nn.softmax(x, axis=axis)
def _gelu(x):
    return jax.nn.gelu(x, approximate=True)
def _silu(x):
    return jax.nn.silu(x)
def _sigmoid(x):
    return jax.nn.sigmoid(x)
def _layernorm(x, axis=-1, eps=1e-5):
    m = jnp.mean(x, axis=axis, keepdims=True)
    v = jnp.var(x, axis=axis, keepdims=True)
    return (x - m) / jnp.sqrt(v + eps)
def _scatter_add(tgt, idx, src, axis=0):
    return tgt.at[idx].add(src)
def _segment_sum(src, seg, n):
    return jax.ops.segment_sum(src, seg, n)
class _Rng:
    def __init__(self, key):
        self._k = key
    def _next(self):
        self._k, sub = jax.random.split(self._k)
        return sub
    def normal(self, shape):
        return jax.random.normal(self._next(), shape, dtype=jnp.bfloat16)
    def randint(self, lo, hi, shape):
        return jax.random.randint(self._next(), shape, lo, hi, dtype=jnp.int32)
    def uniform(self, shape, lo=0.0, hi=1.0):
        return jax.random.uniform(self._next(), shape, jnp.bfloat16, lo, hi)
    def permutation(self, n):
        return jax.random.permutation(self._next(), n)


kernel_name = 'interleave_layers__gqa_block_cached__dense_activation_mish__decode'

def setup_inputs():
    _rng = _Rng(jax.random.key(int.from_bytes(__import__("os").urandom(4), "little")))
    _w = (lambda a: (lambda t: t.astype(jnp.bfloat16) if jnp.issubdtype(t.dtype, jnp.floating) else t)(jnp.asarray(a)))
    def _A_setup():
        B, Sq, D = 1, 1, 512
        Hq, Hkv, Sk, Dh = 32, 8, 65536, 128
        assert Hq % Hkv == 0, (Hq, Hkv)
        return {
            "x": _w((lambda *s: _rng.normal(s) * 0.05)(B, Sq, D)),
            "k_cache": _w((lambda *s: _rng.normal(s) * 1.6)(B, Hkv, Sk, Dh)),
            "v_cache": _w((lambda *s: _rng.normal(s) * 1.6)(B, Hkv, Sk, Dh)),
            "wq": _w((lambda *s: _rng.normal(s) * 1.6)(D, Hq * Dh) * (D ** -0.5)),
            "wo": _w((lambda *s: _rng.normal(s) * 1.6)(Hq * Dh, D) * ((Hq * Dh) ** -0.5)),
        }
    _A_in = _A_setup()

    def _B_setup():
        B, S, D, F = 1, 1, 512, 1792
        return {
            "x": _w((lambda *s: _rng.normal(s) * 0.05)(B, S, D)),
            "w1": _w((lambda *s: _rng.normal(s) * 0.8)(D, F) * (D ** -0.5)),
            "b1": _w((lambda *s: _rng.normal(s) * 0.8)(F)),
            "w2": _w((lambda *s: _rng.normal(s) * 0.8)(F, D) * (F ** -0.5)),
        }
    _B_in = _B_setup()

    return {
        "A_x": _A_in["x"],
        "A_k_cache": _A_in["k_cache"],
        "A_v_cache": _A_in["v_cache"],
        "A_wq": _A_in["wq"],
        "A_wo": _A_in["wo"],
        "B_x": _B_in["x"],
        "B_w1": _B_in["w1"],
        "B_b1": _B_in["b1"],
        "B_w2": _B_in["w2"],
    }

def reference(A_x, A_k_cache, A_v_cache, A_wq, A_wo, B_x, B_w1, B_b1, B_w2):
    def _A_ref(x, k_cache, v_cache, wq, wo):
        B, Sq, D = x.shape
        Hq, Dh = 32, 128
        Hkv = k_cache.shape[1]
        rep = Hq // Hkv
        q = (lambda x, *d: x.transpose(*d))((x @ wq).reshape(B, Sq, Hq, Dh), 0, 2, 1, 3)
        k = jnp.repeat(k_cache, rep, axis=1)
        v = jnp.repeat(v_cache, rep, axis=1)
        scores = jnp.einsum("bhqd,bhkd->bhqk", q, k) * (Dh ** -0.5)
        p = _softmax(scores, axis=-1)
        o = jnp.einsum("bhqk,bhkd->bhqd", p, v)
        return (lambda x, *d: x.transpose(*d))(o, 0, 2, 1, 3).reshape(B, Sq, Hq * Dh) @ wo

    def _B_ref(x, w1, b1, w2):
        h = jnp.einsum("bsd,df->bsf", x, w1) + b1
        sp = jnp.log1p(jnp.exp(-jnp.abs(h))) + jnp.where(h > 0, h, jnp.zeros_like(h))
        act = h * jnp.tanh(sp)
        return jnp.einsum("bsf,fd->bsd", act, w2)

    x = A_x
    x = x + _A_ref(_layernorm(x, axis=-1), A_k_cache, A_v_cache, A_wq, A_wo)
    x = x + _B_ref(_layernorm(x, axis=-1), B_w1, B_b1, B_w2)
    x = x + _A_ref(_layernorm(x, axis=-1), A_k_cache, A_v_cache, A_wq, A_wo)
    x = x + _B_ref(_layernorm(x, axis=-1), B_w1, B_b1, B_w2)
    return x
```

```python
import math

import jax
import jax.numpy as jnp
from jax import lax
import jax.experimental.pallas as pl
import jax.experimental.pallas.tpu as pltpu

D_MODEL = 512
HQ, HKV, DH = 32, 8, 128
REP = HQ // HKV
FF = 1792
EPS = 1e-5

_NT = (((1,), (1,)), ((), ()))
F32 = jnp.float32
BF16 = jnp.bfloat16


def _layernorm(x):
    m = jnp.mean(x, axis=1, keepdims=True)
    xc = x - m
    v = jnp.mean(xc * xc, axis=1, keepdims=True)
    return xc * lax.rsqrt(v + EPS)


def _mish(h):
    sp = jnp.log1p(jnp.exp(-jnp.abs(h))) + jnp.maximum(h, 0.0)
    return h * jnp.tanh(sp)


def make_kernel(SK, BS, NS, D1, D2):
    BPH = SK // BS
    N = HKV * BPH
    NRES = NS
    NSTR = N - NS
    assert NS <= N and D1 <= NS and D2 <= NS and NRES - D2 <= NSTR
    NSEM = max(D1, D2)
    C = (DH ** -0.5) * math.log2(math.e)

    def kernel(x_ref, b1_ref, k_hbm, v_hbm, wq_hbm, wo_hbm, w1_hbm, w2_hbm, o_ref,
               kbuf, vbuf, wq_s, wo_s, w1_s, w2_s, y_s, q_s, m_s, l_s, acc_s, xa_s, cnt_s,
               kv_sem, w_sem):
        def kv_copies(blk, slot, sem):
            h = blk // BPH
            c = blk % BPH
            rows = pl.ds(pl.multiple_of(c * BS, BS), BS)
            return (pltpu.make_async_copy(k_hbm.at[h, rows, :], kbuf.at[slot], kv_sem.at[sem]),
                    pltpu.make_async_copy(v_hbm.at[h, rows, :], vbuf.at[slot], kv_sem.at[sem]))

        def kv_start(blk, slot, sem):
            ck, cv = kv_copies(blk, slot, sem)
            ck.start()
            cv.start()

        def kv_wait(slot, sem):
            ck, cv = kv_copies(0, slot, sem)
            ck.wait()
            cv.wait()

        w_copies = [
            pltpu.make_async_copy(wq_hbm, wq_s, w_sem.at[0]),
            pltpu.make_async_copy(wo_hbm, wo_s, w_sem.at[1]),
            pltpu.make_async_copy(w1_hbm, w1_s, w_sem.at[2]),
            pltpu.make_async_copy(w2_hbm, w2_s, w_sem.at[3]),
        ]
        w_copies[0].start()
        for t in range(2):
            kv_start(t, t % NS, t % D1)
        w_copies[1].start()
        for t in range(2, D1):
            kv_start(t, t % NS, t % D1)
        w_copies[2].start()
        w_copies[3].start()

        row = lax.broadcasted_iota(jnp.int32, (8, DH), 0)

        def reset_state():
            m_s[...] = jnp.full(m_s.shape, -1e30, F32)
            l_s[...] = jnp.zeros(l_s.shape, F32)
            acc_s[...] = jnp.zeros(acc_s.shape, F32)
            xa_s[...] = jnp.zeros(xa_s.shape, F32)
            for h in range(HKV):
                cnt_s[h] = 0

        def make_q(h):
            cols = pl.ds(pl.multiple_of(h * REP * DH, REP * DH), REP * DH)
            qf = jnp.dot(y_s[...], wq_s[:, cols], preferred_element_type=F32)
            q = jnp.zeros((8, DH), F32)
            for r in range(REP):
                q = jnp.where(row == r, qf[:, r * DH:(r + 1) * DH], q)
            q_s[h] = q.astype(BF16)

        def finish_head(h):
            l = jnp.sum(l_s[h], axis=1, keepdims=True)
            o = acc_s[h] / l
            xa = xa_s[...]
            for r in range(REP):
                lhs = jnp.where(row == r, o, 0.0).astype(BF16)
                rows = pl.ds(pl.multiple_of((h * REP + r) * DH, DH), DH)
                xa = xa + jnp.dot(lhs, wo_s[rows, :], preferred_element_type=F32)
            xa_s[...] = xa

        def attend(slot, h):
            cnt = cnt_s[h]

            @pl.when(cnt == 0)
            def _():
                make_q(h)

            q = q_s[h]
            k = kbuf[slot]
            s = lax.dot_general(q, k, _NT, preferred_element_type=F32)
            nt = BS // 128
            mx = s[:, 0:128]
            for t in range(1, nt):
                mx = jnp.maximum(mx, s[:, t * 128:(t + 1) * 128])
            m_old = m_s[h]
            m_new = jnp.maximum(m_old, jnp.max(mx, axis=1, keepdims=True))
            alpha = jnp.exp2((m_old - m_new) * C)
            mc = m_new * C
            ps = [jnp.exp2(s[:, t * 128:(t + 1) * 128] * C - mc) for t in range(nt)]
            ls = ps[0]
            for t in range(1, nt):
                ls = ls + ps[t]
            p = jnp.concatenate(ps, axis=1).astype(BF16)
            pv = jnp.dot(p, vbuf[slot], preferred_element_type=F32)
            m_s[h] = m_new
            l_s[h] = alpha * l_s[h] + ls
            acc_s[h] = alpha * acc_s[h] + pv
            cnt_s[h] = cnt + 1

            @pl.when(cnt == BPH - 1)
            def _():
                finish_head(h)

        def after_attention(x):
            attn = jnp.sum(xa_s[...], axis=0, keepdims=True)
            x = x + attn
            y = _layernorm(x).astype(BF16)
            hid = jnp.dot(y, w1_s[...], preferred_element_type=F32) + b1_ref[...].astype(F32)
            act = _mish(hid).astype(BF16)
            return x + jnp.dot(act, w2_s[...], preferred_element_type=F32)

        x = jnp.broadcast_to(x_ref[...].astype(F32), (8, D_MODEL))
        y_s[...] = _layernorm(x).astype(BF16)
        reset_state()
        w_copies[0].wait()
        w_copies[1].wait()

        def pass1(t, carry):
            kv_wait(t % NS, t % D1)

            @pl.when(t + D1 < N)
            def _():
                kv_start(t + D1, (t + D1) % NS, t % D1)

            attend(t % NS, t // BPH)
            return carry

        lax.fori_loop(0, N, pass1, 0)
        w_copies[2].wait()
        w_copies[3].wait()
        x = after_attention(x)
        y_s[...] = _layernorm(x).astype(BF16)
        reset_state()

        def res_slot(i):
            return (N - NS + i) % NS

        def prologue(i, carry):
            attend(res_slot(i), (N - NS + i) // BPH)
            kv_start(i, res_slot(i), i % D2)
            return carry

        lax.fori_loop(0, D2, prologue, 0)

        def pass2(s, carry):
            @pl.when(s < NRES - D2)
            def _():
                attend(res_slot(D2 + s), (N - NS + D2 + s) // BPH)

            slot = res_slot(s % D2)
            kv_wait(slot, s % D2)
            attend(slot, s // BPH)

            @pl.when(s + D2 < NSTR)
            def _():
                kv_start(s + D2, slot, s % D2)

            return carry

        lax.fori_loop(0, NSTR, pass2, 0)
        x = after_attention(x)
        o_ref[...] = x[0:1, :].astype(o_ref.dtype)

    scratch = [
        pltpu.VMEM((NS, BS, DH), BF16),
        pltpu.VMEM((NS, BS, DH), BF16),
        pltpu.VMEM((D_MODEL, HQ * DH), BF16),
        pltpu.VMEM((HQ * DH, D_MODEL), BF16),
        pltpu.VMEM((D_MODEL, FF), BF16),
        pltpu.VMEM((FF, D_MODEL), BF16),
        pltpu.VMEM((8, D_MODEL), BF16),
        pltpu.VMEM((HKV, 8, DH), BF16),
        pltpu.VMEM((HKV, 8, DH), F32),
        pltpu.VMEM((HKV, 8, DH), F32),
        pltpu.VMEM((HKV, 8, DH), F32),
        pltpu.VMEM((8, D_MODEL), F32),
        pltpu.SMEM((HKV,), jnp.int32),
        pltpu.SemaphoreType.DMA((NSEM,)),
        pltpu.SemaphoreType.DMA((4,)),
    ]
    return kernel, scratch


@jax.jit
def pallas_interleave_layers__gqa_block_cached__dense_activation_mish__decode_kernel(
    A_x, A_k_cache, A_v_cache, A_wq, A_wo, B_x, B_w1, B_b1, B_w2,
):
    SK = A_k_cache.shape[2]
    kernel, scratch = make_kernel(SK, 2048, 116, 8, 6)
    vm = pl.BlockSpec(memory_space=pltpu.VMEM)
    hbm = pl.BlockSpec(memory_space=pl.ANY)
    out = pl.pallas_call(
        kernel,
        in_specs=[vm, vm, hbm, hbm, hbm, hbm, hbm, hbm],
        out_specs=vm,
        out_shape=jax.ShapeDtypeStruct((1, D_MODEL), A_x.dtype),
        scratch_shapes=scratch,
        compiler_params=pltpu.CompilerParams(vmem_limit_bytes=128 * 2**20),
    )(A_x.reshape(1, D_MODEL), B_b1.reshape(1, FF), A_k_cache[0], A_v_cache[0], A_wq, A_wo, B_w1, B_w2)
    return out.reshape(1, 1, D_MODEL)
```

```python
import math

import numpy as np
import jax
import jax.numpy as jnp
from jax import lax
import jax.experimental.pallas as pl
import jax.experimental.pallas.tpu as pltpu

D_MODEL = 512
HQ, HKV, DH = 32, 8, 128
REP = HQ // HKV
FF = 1792
EPS = 1e-5

F32 = jnp.float32
BF16 = jnp.bfloat16
U32 = jnp.uint32
_NT = (((1,), (1,)), ((), ()))

TILE_RAW = 64
TILE_PK = 48


def _u(v):
    return np.uint32(v)


def _shl(x, n):
    return lax.shift_left(x, _u(n))


def _shr(x, n):
    return lax.shift_right_logical(x, _u(n))


def _pack4(x0, x1, x2, x3, base):
    u0, u1, u2, u3 = x0 - base, x1 - base, x2 - base, x3 - base
    bad = (u0 | u1) | (u2 | u3)
    w0 = u0 | _shl(u3 & _u(0x000F000F), 11)
    w1 = u1 | _shl(u3 & _u(0x00F000F0), 7)
    w2 = u2 | (_shl(u3 & _u(0x07000700), 3) | (_shr(u3, 1) & _u(0x40004000)))
    return w0, w1, w2, bad


def _unpack4(w0, w1, w2, base):
    keep = _u(0x87FF87FF)
    a = _shr(w0, 11) & _u(0x000F000F)
    b = _shr(w1, 7) & _u(0x00F000F0)
    c = (_shr(w2, 3) & _u(0x07000700)) | (_shl(w2, 1) & _u(0x80008000))
    return (w0 & keep) + base, (w1 & keep) + base, (w2 & keep) + base, ((a | b) | c) + base


def _layernorm(x):
    xc = x - jnp.mean(x, axis=1, keepdims=True)
    return xc * lax.rsqrt(jnp.mean(xc * xc, axis=1, keepdims=True) + EPS)


def _mish(h):
    sp = jnp.log1p(jnp.exp(-jnp.abs(h))) + jnp.maximum(h, 0.0)
    return h * jnp.tanh(sp)


def make_kernel(SK, BS, CAP, NSTG, CH, SM):
    BPH = SK // BS
    N = HKV * BPH
    NT = BS // DH
    HALF = 2048
    NW = 12
    W_TILES = [(16, 16)] * 8 + [(16, 12)] * 2 + [(14, 14)] * 2
    assert BS <= HALF and NW % NSTG == 0 and NSTG < N and CAP % 8 == 0
    assert CAP >= sum(a + b for a, b in W_TILES) * TILE_RAW
    SCALE = (DH ** -0.5) * math.log2(math.e)
    S_OFF, S_NA, S_FULL, S_SKIP, S_E0, S_E1, S_IA, S_IS, S_ACC, S_ISSUE = range(10)

    def kernel(x_ref, b1_hbm, k_hbm, v_hbm, wq_hbm, wo_hbm, w1_hbm, w2_hbm, o_ref,
               stg_s, arena_s, b1_s, y_s, q_s, m_s, l_s, acc_s, xa_s,
               cnt_s, st_s, tab_s, stg_sem, b1_sem):

        def kv_copies(blk, slot):
            h = blk // BPH
            rows = pl.ds(pl.multiple_of((blk % BPH) * BS, BS), BS)
            return [pltpu.make_async_copy(src.at[h, rows, :], stg_s.at[slot, part, pl.ds(0, BS), :], stg_sem.at[slot])
                    for part, src in enumerate((k_hbm, v_hbm))]

        def kv_start(blk, slot):
            for c in kv_copies(blk, slot):
                c.start()

        def kv_wait(slot):
            for c in kv_copies(0, slot):
                c.wait()

        def weight_copies(u):
            slot = u % NSTG
            out = []

            def add(src, part, row, n):
                out.append(pltpu.make_async_copy(src, stg_s.at[slot, part, pl.ds(row, n), :], stg_sem.at[slot]))

            if u < 4:
                for j in range(8):
                    c = (8 * u + j) * DH
                    add(wq_hbm.at[:, pl.ds(c, DH)], j // 4, (j % 4) * D_MODEL, D_MODEL)
            elif u < 8:
                for j in range(8):
                    r = (2 * (u - 4) + j // 4) * REP * DH
                    add(wo_hbm.at[pl.ds(r, REP * DH), pl.ds((j % 4) * DH, DH)], j // 4, (j % 4) * D_MODEL, D_MODEL)
            elif u < 10:
                for j in range(7):
                    c = (7 * (u - 8) + j) * DH
                    add(w1_hbm.at[:, pl.ds(c, DH)], j // 4, (j % 4) * D_MODEL, D_MODEL)
            else:
                for j in range(2):
                    c = (2 * (u - 10) + j) * DH
                    add(w2_hbm.at[:, pl.ds(c, DH)], j, 0, FF)
            return out

        def start_unit(u):
            if u < NW:
                for c in weight_copies(u):
                    c.start()
            else:
                kv_start(u - NW, u % NSTG)

        for u in range(NSTG):
            start_unit(u)
        b1_copy = pltpu.make_async_copy(b1_hbm, b1_s, b1_sem.at[0])
        b1_copy.start()

        def arena_vreg(off, i):
            return arena_s[pl.ds(pl.multiple_of(off + 8 * i, 8), 8), :]

        def stg_vreg(slot, part, i):
            return pltpu.bitcast(stg_s[slot, part, pl.ds(pl.multiple_of(16 * i, 16), 16), :], U32)

        def base_vec(e0):
            b = lax.shift_left(e0, 7)
            b = b | lax.shift_left(b, 16)
            return lax.bitcast_convert_type(jnp.full((8, DH), b, jnp.int32), U32)

        def window(slot, part):
            mag = _u(0x7FFF0000)
            mx = None
            for i in range(8):
                x = stg_vreg(slot, part, i)
                t = jnp.maximum(pltpu.bitcast(x & mag, F32), pltpu.bitcast(_shl(x, 16) & mag, F32))
                mx = t if mx is None else jnp.maximum(mx, t)
            top = jnp.max(jnp.max(mx, axis=1, keepdims=True), axis=0, keepdims=True)
            e = lax.shift_right_logical(pltpu.bitcast(top, jnp.int32), 23)[0, 0]
            return jnp.clip(e - 14, 0, 240)

        def pack_half(slot, part, ntiles, dst, e0, unroll):
            base = base_vec(e0)

            def two_tiles(i, bad):
                for g in range(4):
                    *ws, b = _pack4(*(stg_vreg(slot, part, 16 * i + 4 * g + r) for r in range(4)), base)
                    for r, w in enumerate(ws):
                        arena_s[pl.ds(pl.multiple_of(dst + 8 * (12 * i + 3 * g + r), 8), 8), :] = w
                    bad = bad | b
                return bad

            return lax.fori_loop(0, ntiles // 2, two_tiles, jnp.zeros((8, DH), U32), unroll=unroll)

        def copy_half(slot, part, ntiles, dst):
            def two_tiles(i, c):
                for r in range(16):
                    arena_s[pl.ds(pl.multiple_of(dst + 8 * (16 * i + r), 8), 8), :] = stg_vreg(slot, part, 16 * i + r)
                return c

            lax.fori_loop(0, ntiles // 2, two_tiles, 0)

        def retain(slot, nt0, nt1, unroll, backoff):
            off = st_s[S_OFF]
            na = st_s[S_NA]
            skip = st_s[S_SKIP]
            open_ = st_s[S_FULL] == 0
            st_s[S_E0] = -1
            st_s[S_E1] = -1
            st_s[S_SKIP] = jnp.maximum(skip - 1, 0)

            @pl.when(jnp.logical_and(jnp.logical_and(open_, skip == 0), off + (nt0 + nt1) * TILE_PK <= CAP))
            def _():
                e0 = window(slot, 0)
                e1 = window(slot, 1)
                bad = pack_half(slot, 0, nt0, off, e0, unroll) | pack_half(slot, 1, nt1, off + nt0 * TILE_PK, e1, unroll)
                bad = jnp.where((bad & _u(0x78007800)) != 0, 1.0, 0.0)
                ok = jnp.max(jnp.max(bad, axis=1, keepdims=True), axis=0, keepdims=True)[0, 0] == 0.0
                st_s[S_E0] = jnp.where(ok, e0, -1)
                st_s[S_E1] = jnp.where(ok, e1, -1)
                st_s[S_SKIP] = jnp.where(ok, 0, backoff)

            packed = st_s[S_E0] >= 0
            raw = jnp.logical_and(jnp.logical_not(packed),
                                  jnp.logical_and(open_, off + (nt0 + nt1) * TILE_RAW <= CAP))

            @pl.when(raw)
            def _():
                copy_half(slot, 0, nt0, off)
                copy_half(slot, 1, nt1, off + nt0 * TILE_RAW)

            kept = jnp.logical_or(packed, raw)

            @pl.when(kept)
            def _():
                tab_s[0, na] = off
                tab_s[1, na] = st_s[S_E0]
                tab_s[2, na] = st_s[S_E1]
                st_s[S_NA] = na + 1
                st_s[S_OFF] = off + (nt0 + nt1) * jnp.where(packed, TILE_PK, TILE_RAW)

            st_s[S_FULL] = jnp.where(kept, 0, 1)

        def raw_tiles(off, t0, n):
            return pltpu.bitcast(arena_s[pl.ds(pl.multiple_of(off + t0 * TILE_RAW, 8), n * TILE_RAW), :], BF16)

        def packed_tiles(off, t0, n, base):
            xs = []
            for g in range(2 * n):
                xs.extend(_unpack4(*(arena_vreg(off + t0 * TILE_PK, 3 * g + i) for i in range(3)), base))
            return pltpu.bitcast(jnp.concatenate(xs, axis=0), BF16)

        def with_tiles(entry, half, nt0, fn):
            off = tab_s[0, entry]
            e = tab_s[1 + half, entry]

            def raw():
                return fn(lambda t0, n: raw_tiles(off + half * nt0 * TILE_RAW, t0, n))

            return lax.cond(e < 0, raw, lambda: with_packed_tiles(entry, half, nt0, fn))

        def with_packed_tiles(entry, half, nt0, fn):
            off = tab_s[0, entry]
            base = base_vec(tab_s[1 + half, entry])
            return fn(lambda t0, n: packed_tiles(off + half * nt0 * TILE_PK, t0, n, base))

        row = lax.broadcasted_iota(jnp.int32, (8, DH), 0)
        row8 = lax.broadcasted_iota(jnp.int32, (8, D_MODEL), 0)

        def reset_state(x):
            m_s[...] = jnp.full(m_s.shape, -1e30, F32)
            l_s[...] = jnp.zeros(l_s.shape, F32)
            acc_s[...] = jnp.zeros(acc_s.shape, F32)
            xa_s[...] = jnp.where(row8 == 0, x, 0.0)
            y_s[...] = _layernorm(x).astype(BF16)
            for h in range(HKV):
                cnt_s[h] = 0

        def make_q(h):
            y = y_s[...]

            def project(tiles):
                q = jnp.zeros((8, DH), F32)
                for r in range(REP):
                    qr = jnp.dot(y, tiles(4 * r, 4), preferred_element_type=F32)
                    q = jnp.where(row % REP == r, qr, q)
                return q

            q_s[h] = with_tiles(h // 2, h % 2, 16, project).astype(BF16)

        def finish_head(h):
            o = acc_s[h // 2] / jnp.sum(l_s[h // 2], axis=1, keepdims=True)
            lhs = jnp.concatenate([jnp.where(row == REP * (h % 2) + r, o, 0.0) for r in range(REP)], axis=1).astype(BF16)

            def project(tiles):
                return jnp.concatenate(
                    [jnp.dot(lhs, tiles(4 * n, 4), preferred_element_type=F32) for n in range(D_MODEL // DH)], axis=1)

            xa_s[...] += with_tiles(4 + h // 2, h % 2, 16, project)

        def attend(h, k_tiles, v_tiles):
            q = q_s[h]
            tpc = CH // DH
            cps = SM // CH
            ss = []
            for c in range(BS // CH):
                s = lax.dot_general(q, k_tiles(c * tpc, tpc), _NT, preferred_element_type=F32)
                ss.extend(s[:, t * DH:(t + 1) * DH] for t in range(tpc))
            m_old, l_old, acc_old = m_s[h // 2], l_s[h // 2], acc_s[h // 2]
            m, l, acc = m_old, l_old, acc_old
            for g in range(BS // SM):
                tiles = ss[g * cps * tpc:(g + 1) * cps * tpc]
                mx = tiles[0]
                for t in tiles[1:]:
                    mx = jnp.maximum(mx, t)
                m_new = jnp.maximum(m, jnp.max(mx, axis=1, keepdims=True))
                alpha = jnp.exp2((m - m_new) * SCALE)
                mc = m_new * SCALE
                ps = [jnp.exp2(t * SCALE - mc) for t in tiles]
                ls = ps[0]
                for p in ps[1:]:
                    ls = ls + p
                pv = None
                for i in range(cps):
                    p = jnp.concatenate(ps[i * tpc:(i + 1) * tpc], axis=1).astype(BF16)
                    d = jnp.dot(p, v_tiles((g * cps + i) * tpc, tpc), preferred_element_type=F32)
                    pv = d if pv is None else pv + d
                l = alpha * l + ls
                acc = alpha * acc + pv
                m = m_new
            own = row // REP == h % 2
            m_s[h // 2] = jnp.where(own, m, m_old)
            l_s[h // 2] = jnp.where(own, l, l_old)
            acc_s[h // 2] = jnp.where(own, acc, acc_old)

        def mlp_with(x, reader):
            y = _layernorm(x).astype(BF16)
            hid = []
            for p in range(2):
                for half, ncol in ((0, 4), (1, 3)):
                    hid.append(reader(8 + p, half, 16, lambda tiles: jnp.concatenate(
                        [jnp.dot(y, tiles(4 * j, 4), preferred_element_type=F32) for j in range(ncol)], axis=1)))
            hid = jnp.concatenate(hid, axis=1) + b1_s[...].astype(F32).reshape(1, FF)
            act = _mish(hid).astype(BF16)

            def down(tiles):
                out = None
                for t0, n in ((0, 4), (4, 4), (8, 4), (12, 2)):
                    d = jnp.dot(act[:, t0 * DH:(t0 + n) * DH], tiles(t0, n), preferred_element_type=F32)
                    out = d if out is None else out + d
                return out

            return x + jnp.concatenate([reader(10 + p, half, 14, down) for p in range(2) for half in range(2)], axis=1)

        def mlp(x):
            all_packed = jnp.minimum(jnp.minimum(tab_s[1, 8], tab_s[1, 9]), jnp.minimum(tab_s[1, 10], tab_s[1, 11])) >= 0
            return lax.cond(all_packed, lambda: mlp_with(x, with_packed_tiles), lambda: mlp_with(x, with_tiles))

        for i in (S_OFF, S_NA, S_FULL, S_SKIP, S_IA, S_IS, S_ACC, S_ISSUE):
            st_s[i] = 0
        reset_state(jnp.broadcast_to(x_ref[...].astype(F32), (8, D_MODEL)))
        for u in range(NW):
            for c in weight_copies(u):
                c.wait()
            retain(u % NSTG, *W_TILES[u], unroll=1, backoff=0)
            start_unit(u + NSTG)
        b1_copy.wait()


        def head_begin(h):
            @pl.when(cnt_s[h] == 0)
            def _():
                make_q(h)

        def head_end(h):
            cnt = cnt_s[h]
            cnt_s[h] = cnt + 1

            @pl.when(cnt == BPH - 1)
            def _():
                finish_head(h)

        def attend_staged(h, slot):
            attend(h, lambda t0, n: stg_s[slot, 0, t0 * DH:(t0 + n) * DH, :],
                   lambda t0, n: stg_s[slot, 1, t0 * DH:(t0 + n) * DH, :])

        def residual():
            return jnp.broadcast_to(jnp.sum(xa_s[...], axis=0, keepdims=True), (8, D_MODEL))

        def layer1(j, carry):
            slot = j % NSTG
            h = j // BPH
            head_begin(h)
            kv_wait(slot)
            attend_staged(h, slot)

            @pl.when(j < N - NSTG)
            def _():
                retain(slot, NT, NT, unroll=4, backoff=7)
                kv_start(j + NSTG, slot)

            head_end(h)
            return carry

        lax.fori_loop(0, N, layer1, 0)
        reset_state(mlp(residual()))

        na = st_s[S_NA] - NW
        nstr = N - NSTG - na
        st_s[S_ACC] = 3 * na

        def layer2(j, carry):
            ia, i_s, acc = st_s[S_IA], st_s[S_IS], st_s[S_ACC]
            is_tail = j < NSTG
            later = j >= NSTG
            is_arena = jnp.logical_and(
                later, jnp.logical_and(ia < na, jnp.logical_or(acc >= nstr, i_s >= nstr)))
            is_str = jnp.logical_and(later, jnp.logical_not(is_arena))
            blk = jnp.where(is_tail, N - NSTG + j, jnp.where(is_arena, ia, na + i_s))
            slot = jnp.where(is_str, N - NSTG + i_s, blk) % NSTG
            h = blk // BPH
            head_begin(h)

            @pl.when(is_str)
            def _():
                kv_wait(slot)

            @pl.when(jnp.logical_not(is_arena))
            def _():
                attend_staged(h, slot)

            @pl.when(is_arena)
            def _():
                off = tab_s[0, NW + ia]
                e0 = tab_s[1, NW + ia]
                e1 = tab_s[2, NW + ia]

                @pl.when(e0 < 0)
                def _():
                    attend(h, lambda t0, n: raw_tiles(off, t0, n), lambda t0, n: raw_tiles(off + NT * TILE_RAW, t0, n))

                @pl.when(e0 >= 0)
                def _():
                    b0, b1 = base_vec(e0), base_vec(e1)
                    attend(h, lambda t0, n: packed_tiles(off, t0, n, b0),
                           lambda t0, n: packed_tiles(off + NT * TILE_PK, t0, n, b1))

            issue = st_s[S_ISSUE]

            @pl.when(jnp.logical_and(jnp.logical_not(is_arena), issue < nstr))
            def _():
                kv_start(na + issue, slot)
                st_s[S_ISSUE] = issue + 1

            st_s[S_IA] = ia + jnp.where(is_arena, 1, 0)
            st_s[S_IS] = i_s + jnp.where(is_str, 1, 0)
            st_s[S_ACC] = acc + jnp.where(is_str, na, 0) - jnp.where(is_arena, nstr, 0)
            head_end(h)
            return carry

        lax.fori_loop(0, N, layer2, 0)
        o_ref[...] = mlp(residual())[0:1, :].astype(o_ref.dtype)

    scratch = [
        pltpu.VMEM((NSTG, 2, HALF, DH), BF16),
        pltpu.VMEM((CAP, DH), U32),
        pltpu.VMEM((FF,), BF16),
        pltpu.VMEM((8, D_MODEL), BF16),
        pltpu.VMEM((HKV, 8, DH), BF16),
        pltpu.VMEM((HKV // 2, 8, DH), F32),
        pltpu.VMEM((HKV // 2, 8, DH), F32),
        pltpu.VMEM((HKV // 2, 8, DH), F32),
        pltpu.VMEM((8, D_MODEL), F32),
        pltpu.SMEM((HKV,), jnp.int32),
        pltpu.SMEM((16,), jnp.int32),
        pltpu.SMEM((3, NW + N), jnp.int32),
        pltpu.SemaphoreType.DMA((NSTG,)),
        pltpu.SemaphoreType.DMA((1,)),
    ]
    return kernel, scratch


BS = 2048
CAP_KB = 127872
NSTG = 3
CH = 512
SM = 512
vmem_mb = 128


@jax.jit
def pallas_interleave_layers__gqa_block_cached__dense_activation_mish__decode_kernel(A_x, A_k_cache, A_v_cache, A_wq, A_wo, B_x, B_w1, B_b1, B_w2):
    SK = A_k_cache.shape[2]
    kernel, scratch = make_kernel(SK, BS, CAP_KB * 2, NSTG, CH, SM)
    vm = pl.BlockSpec(memory_space=pltpu.VMEM)
    hbm = pl.BlockSpec(memory_space=pl.ANY)
    out = pl.pallas_call(
        kernel,
        in_specs=[vm, hbm, hbm, hbm, hbm, hbm, hbm, hbm],
        out_specs=vm,
        out_shape=jax.ShapeDtypeStruct((1, D_MODEL), A_x.dtype),
        scratch_shapes=scratch,
        compiler_params=pltpu.CompilerParams(vmem_limit_bytes=vmem_mb * 2**20),
    )(A_x.reshape(1, D_MODEL), B_b1, A_k_cache[0], A_v_cache[0], A_wq, A_wo, B_w1, B_w2)
    return out.reshape(1, 1, D_MODEL)
```
